```python
import jax
import jax.numpy as jnp

def _softmax(x, axis=-1):
    return jax.nn.softmax(x, axis=axis)
def _gelu(x):
    return jax.nn.gelu(x, approximate=True)
def _silu(x):
    return jax.nn.silu(x)
def _sigmoid(x):
    return jax.nn.sigmoid(x)
def _layernorm(x, axis=-1, eps=1e-5):
    m = jnp.mean(x, axis=axis, keepdims=True)
    v = jnp.var(x, axis=axis, keepdims=True)
    return (x - m) / jnp.sqrt(v + eps)
def _scatter_add(tgt, idx, src, axis=0):
    return tgt.at[idx].add(src)
def _segment_sum(src, seg, n):
    return jax.ops.segment_sum(src, seg, n)
class _Rng:
    def __init__(self, key):
        self._k = key
    def _next(self):
        self._k, sub = jax.random.split(self._k)
        return sub
    def normal(self, shape):
        return jax.random.normal(self._next(), shape, dtype=jnp.bfloat16)
    def randint(self, lo, hi, shape):
        return jax.random.randint(self._next(), shape, lo, hi, dtype=jnp.int32)
    def uniform(self, shape, lo=0.0, hi=1.0):
        return jax.random.uniform(self._next(), shape, jnp.bfloat16, lo, hi)
    def permutation(self, n):
        return jax.random.permutation(self._next(), n)


kernel_name = 'gated_mix__linear_kernel_hedgehog__moe_arch_mod__prompt'

def setup_inputs():
    _rng = _Rng(jax.random.key(int.from_bytes(__import__("os").urandom(4), "little")))
    _w = (lambda a: (lambda t: t.astype(jnp.bfloat16) if jnp.issubdtype(t.dtype, jnp.floating) else t)(jnp.asarray(a)))
    def _A_setup():
        B, S, D, H = 1, 2048, 1024, 32
        Dh = D // H
        return {
            "x": _w((lambda *s: _rng.normal(s) * 0.05)(B, S, D)),
            "wqkv": _w((lambda *s: _rng.normal(s) * 0.05)(D, 3 * D)),
            "w_phi": _w((lambda *s: _rng.normal(s) * 0.05)(H, Dh, Dh) * (Dh ** -0.5)),
            "wo": _w((lambda *s: _rng.normal(s) * 0.05)(D, D)),
        }
    _A_in = _A_setup()

    def _B_setup():
        B, S, D, F, C = 1, 2048, 1024, 3584, 1
        return {
            "x": _w((lambda *s: _rng.normal(s) * 0.05)(B, S, D)),
            "w_r": _w((lambda *s: _rng.normal(s) * 0.05)(D)),
            "w_gate": _w((lambda *s: _rng.normal(s) * 0.05)(D, F)),
            "w_up": _w((lambda *s: _rng.normal(s) * 0.05)(D, F)),
            "w_down": _w((lambda *s: _rng.normal(s) * 0.05)(F, D)),
        }
    _B_in = _B_setup()

    return {
        "A_x": _A_in["x"],
        "A_wqkv": _A_in["wqkv"],
        "A_w_phi": _A_in["w_phi"],
        "A_wo": _A_in["wo"],
        "B_x": _B_in["x"],
        "B_w_r": _B_in["w_r"],
        "B_w_gate": _B_in["w_gate"],
        "B_w_up": _B_in["w_up"],
        "B_w_down": _B_in["w_down"],
        "gate_w": _w((lambda *s: _rng.normal(s) * 0.05)(1024)),
    }

def reference(A_x, A_wqkv, A_w_phi, A_wo, B_x, B_w_r, B_w_gate, B_w_up, B_w_down, gate_w):
    def _A_ref(x, wqkv, w_phi, wo):
        B, S, D = x.shape
        H = 32; Dh = D // H
        qkv = (lambda x, *d: x.transpose(*d))((x @ wqkv).reshape(B, S, 3, H, Dh), 2, 0, 3, 1, 4)
        q, k, v = qkv[0], qkv[1], qkv[2]
        pq = jnp.einsum("bhsd,hdf->bhsf", q, w_phi)
        pk = jnp.einsum("bhsd,hdf->bhsf", k, w_phi)
        phi_q = jnp.concatenate([_softmax(pq, axis=-1), _softmax(-pq, axis=-1)], axis=-1)
        phi_k = jnp.concatenate([_softmax(pk, axis=-1), _softmax(-pk, axis=-1)], axis=-1)
        kv = jnp.einsum("bhsf,bhsd->bhfd", phi_k, v)
        z  = jnp.einsum("bhsf->bhf", phi_k)
        num = jnp.einsum("bhqf,bhfd->bhqd", phi_q, kv)
        den = jnp.einsum("bhqf,bhf->bhq", phi_q, z)[..., None] + 1e-6
        o = num / den
        return (lambda x, *d: x.transpose(*d))(o, 0, 2, 1, 3).reshape(B, S, D) @ wo

    def _B_ref(x, w_r, w_gate, w_up, w_down):
        B, S, D = x.shape
        C = 1
        r = x @ w_r
        idx = jnp.argsort(-r, axis=-1)[:, :C]
        idx_e = jnp.repeat(idx.reshape(B, C, 1), D, axis=2)
        x_sel = jnp.take_along_axis(x, idx_e, axis=1)
        g = _silu(x_sel @ w_gate)
        u = x_sel @ w_up
        y = (g * u) @ w_down
        r_sel = _sigmoid(jnp.take_along_axis(r, idx, axis=1))
        y = y * r_sel.reshape(B, C, 1)
        b_off = (jnp.arange(B) * S).reshape(B, 1)
        flat_idx = (idx + b_off).reshape(B * C)
        zero = (x * 0.0).reshape(B * S, D)
        upd = _scatter_add(zero, flat_idx, y.reshape(B * C, D), axis=0)
        return x + upd.reshape(B, S, D)

    x = A_x
    g = _sigmoid((x * gate_w).sum(-1, keepdims=True))
    a = _A_ref(x, A_wqkv, A_w_phi, A_wo)
    b = _B_ref(x, B_w_r, B_w_gate, B_w_up, B_w_down)
    return g * a + (1 - g) * b
```

```python
import functools
import math

import jax
import jax.numpy as jnp
from jax import lax
import jax.experimental.pallas as pl
import jax.experimental.pallas.tpu as pltpu

S, D, H, DH, F = 2048, 1024, 32, 32, 3584
T = 512
NT_ = S // T
NP = H // 2
AUG = 80
LOG2E = math.log2(math.e)
F32, BF16 = jnp.float32, jnp.bfloat16
_NN = (((1,), (0,)), ((), ()))
_NT = (((1,), (1,)), ((), ()))


def _dot(a, b, dn):
    return lax.dot_general(a, b, dn, preferred_element_type=F32)


def _allreduce(v, op):
    v = op(v, pltpu.roll(v, 4, 0))
    return op(v, pltpu.roll(v, 2, 0))


def _phi(p):
    t = p.shape[1]
    p = p.reshape(8, 8, t)
    mx = _allreduce(jnp.max(p, axis=0), jnp.maximum)
    mn = _allreduce(jnp.min(p, axis=0), jnp.minimum)
    ep = jnp.exp2(p - mx[None])
    en = jnp.exp2(mn[None] - p)
    rp = 1.0 / _allreduce(jnp.sum(ep, axis=0), jnp.add)
    rn = 1.0 / _allreduce(jnp.sum(en, axis=0), jnp.add)
    fp = (ep * rp[None]).reshape(64, t).astype(BF16)
    fn = (en * rn[None]).reshape(64, t).astype(BF16)
    return jnp.concatenate([fp, fn], axis=0)


def _sublane_allsum(v):
    v = v + pltpu.roll(v, 4, 0)
    v = v + pltpu.roll(v, 2, 0)
    return v + pltpu.roll(v, 1, 0)


def _matvec(w_ref, col_ref, k0, k1, c0, c1):
    n = (c1 - c0) // 128
    acc = [None] * n
    for k in range(k0, k1, 16):
        xc = col_ref[k:k + 16, :]
        for j in range(n):
            w = w_ref[k:k + 16, c0 + 128 * j:c0 + 128 * (j + 1)].astype(F32) * xc
            w = w[:8] + w[8:]
            acc[j] = w if acc[j] is None else acc[j] + w
    return jnp.concatenate(acc, axis=1)


def _to_col(row8, col_ref, base):
    for j in range(row8.shape[1] // 128):
        blk = jnp.broadcast_to(row8[0:1, 128 * j:128 * (j + 1)], (128, 128))
        col_ref[base + 128 * j:base + 128 * (j + 1), :] = blk.T


def _kernel(x_hbm, wqkv_hbm, wphi_hbm, wo_hbm, wr_ref, wg_hbm, wu_hbm, wd_hbm, gw_ref,
            out_hbm,
            x_v, wqkv_v, wphi_v, wo_v, wg_v, wu_v, wd_v,
            wt_v, kv_v, kvm_v, ot_v, r_v, xcol_v, hcol_v, out_v,
            sems, osems):
    copies = {}

    def start(name, src, dst):
        c = pltpu.make_async_copy(src, dst, sems.at[len(copies)])
        copies[name] = c
        c.start()

    def rows(i):
        return slice(i * T, (i + 1) * T)

    start("wphi", wphi_hbm, wphi_v)
    start("wk", wqkv_hbm.at[:, D:2 * D], wqkv_v.at[:, D:2 * D])
    start("x0", x_hbm.at[rows(0)], x_v.at[rows(0)])
    start("wv", wqkv_hbm.at[:, 2 * D:3 * D], wqkv_v.at[:, 2 * D:3 * D])
    start("x1", x_hbm.at[rows(1)], x_v.at[rows(1)])
    start("x2", x_hbm.at[rows(2)], x_v.at[rows(2)])
    start("x3", x_hbm.at[rows(3)], x_v.at[rows(3)])
    start("wg", wg_hbm, wg_v)
    start("wu", wu_hbm, wu_v)
    start("wq", wqkv_hbm.at[:, 0:D], wqkv_v.at[:, 0:D])
    start("wd", wd_hbm, wd_v)
    start("wo", wo_hbm, wo_v)

    def prep(src_col, dst_row):
        c = lax.broadcasted_iota(jnp.int32, (128, DH), 0)
        f = lax.broadcasted_iota(jnp.int32, (128, DH), 1)
        sel = jnp.where(((c & 63) >> 1) == f, 1.0, 0.0).astype(BF16)
        c = lax.broadcasted_iota(jnp.int32, (128, 128), 0)
        hd = lax.broadcasted_iota(jnp.int32, (128, 128), 1)
        keep = (((c >> 6) << 1) + (c & 1)) == (hd >> 5)
        for g in range(H // 4):
            wblk = wphi_v[4 * g:4 * g + 4].reshape(128, DH)
            m = jnp.where(keep, _dot(sel, wblk, _NT), 0.0).astype(BF16)
            w = wqkv_v[:, src_col + 128 * g:src_col + 128 * (g + 1)]
            wt_v[dst_row + 128 * g:dst_row + 128 * (g + 1), :] = (
                _dot(m, w, _NT) * LOG2E).astype(BF16)

    def phase1(i):
        xt = x_v[rows(i), :]
        kt = _dot(wt_v[0:D, :], xt, _NT)
        vt = _dot(wt_v[D:2 * D, :], xt, _NT).astype(BF16)
        ones = jnp.ones((AUG - 64, T), BF16)
        for p in range(NP):
            phi = _phi(kt[64 * p:64 * (p + 1)])
            va = jnp.concatenate([vt[64 * p:64 * (p + 1)], ones], axis=0)
            kv = _dot(va, phi, _NT)
            if i == 0:
                kv_v[p] = kv
            else:
                kv_v[p] += kv

    def finish_kv():
        r = lax.broadcasted_iota(jnp.int32, (AUG, 128), 0)
        c = lax.broadcasted_iota(jnp.int32, (AUG, 128), 1)
        head = jnp.where(r < 64, r >> 5, (r - 64) >> 3)
        keep = head == (c & 1)
        for p in range(NP):
            kvm_v[p] = jnp.where(keep, kv_v[p], 0.0).astype(BF16)

    def q_proj(i):
        return _dot(wt_v[2 * D:3 * D, :], x_v[rows(i), :], _NT)

    def attend(i, qt):
        for p in range(NP):
            phi = _phi(qt[64 * p:64 * (p + 1)])
            nd = _dot(kvm_v[p], phi, _NN)
            r0 = 1.0 / (nd[64:72] + 1e-6)
            r1 = 1.0 / (nd[72:80] + 1e-6)
            o0 = (nd[0:32].reshape(4, 8, T) * r0[None]).reshape(32, T)
            o1 = (nd[32:64].reshape(4, 8, T) * r1[None]).reshape(32, T)
            ot_v[64 * p:64 * (p + 1), rows(i)] = jnp.concatenate([o0, o1], axis=0).astype(BF16)

    def route():
        wr = wr_ref[...].astype(F32).reshape(1, D)
        for j in range(S // 128):
            b = x_v[128 * j:128 * (j + 1), :].astype(F32)
            r_v[128 * j:128 * (j + 1), :] = jnp.sum(b * wr, axis=1, keepdims=True)
        r = r_v[...].astype(BF16).astype(F32)
        bits = lax.bitcast_convert_type(jnp.where(r == 0.0, 0.0, r), jnp.int32)
        key = jnp.where(bits < 0, bits ^ 0x7FFFFFFF, bits)
        key = jnp.where(r != r, jnp.iinfo(jnp.int32).min, key)
        pos = lax.broadcasted_iota(jnp.int32, (S, 1), 0)
        idx = jnp.min(jnp.where(key == jnp.max(key), pos, S))
        base = pl.multiple_of((idx >> 4) << 4, 16)
        blk = x_v[pl.ds(base, 16), :].astype(F32)
        sub = lax.broadcasted_iota(jnp.int32, (16, D), 0)
        blk = jnp.where(sub == (idx & 15), blk, 0.0)
        row = _sublane_allsum(blk[:8] + blk[8:])
        _to_col(row, xcol_v, 0)
        r_sel = jnp.sum(row * wr, axis=1, keepdims=True).astype(BF16).astype(F32)
        return idx, jax.nn.sigmoid(r_sel)

    def gate_up(c0, c1):
        g = _sublane_allsum(_matvec(wg_v, xcol_v, 0, D, c0, c1))
        u = _sublane_allsum(_matvec(wu_v, xcol_v, 0, D, c0, c1))
        _to_col(g * jax.nn.sigmoid(g) * u, hcol_v, c0)

    def down():
        return _sublane_allsum(_matvec(wd_v, hcol_v, 0, F, 0, D))

    out_copies = []

    def mix(i, idx, y):
        o = ot_v[:, rows(i)].T
        a = _dot(o, wo_v[...], _NN)
        gw = gw_ref[...].astype(F32).reshape(1, D)
        g = jax.nn.sigmoid(jnp.sum(x_v[rows(i), :].astype(F32) * gw, axis=1, keepdims=True))
        b = x_v[rows(i), :].astype(F32)
        pos = lax.broadcasted_iota(jnp.int32, (T, D), 0) + i * T
        b = b + (b * 0.0 + jnp.where(pos == idx, y, 0.0))
        out_v[rows(i), :] = (g * a + (1.0 - g) * b).astype(BF16)
        c = pltpu.make_async_copy(out_v.at[rows(i)], out_hbm.at[rows(i)], osems.at[i])
        c.start()
        out_copies.append(c)

    copies["wphi"].wait()
    copies["wk"].wait()
    prep(D, 0)
    copies["x0"].wait()
    copies["wv"].wait()
    for g in range(D // 128):
        wt_v[D + 128 * g:D + 128 * (g + 1), :] = wqkv_v[:, 2 * D + 128 * g:2 * D + 128 * (g + 1)].T
    phase1(0)
    copies["x1"].wait()
    copies["x2"].wait()
    copies["x3"].wait()
    phase1(1)
    idx, r_sel = route()
    copies["wg"].wait()
    copies["wu"].wait()
    phase1(2)
    for c in range(0, 4):
        gate_up(512 * c, 512 * (c + 1))
    copies["wq"].wait()
    phase1(3)
    for c in range(4, 7):
        gate_up(512 * c, 512 * (c + 1))
    prep(0, 2 * D)
    finish_kv()
    copies["wd"].wait()
    copies["wo"].wait()
    qt = q_proj(0)
    y = (down() * r_sel)[0:1]
    attend(0, qt)
    for i in range(1, NT_):
        qt = q_proj(i)
        mix(i - 1, idx, y)
        attend(i, qt)
    mix(NT_ - 1, idx, y)
    for c in out_copies:
        c.wait()


@jax.jit
def pallas_gated_mix__linear_kernel_hedgehog__moe_arch_mod__prompt_kernel(
    A_x, A_wqkv, A_w_phi, A_wo, B_x, B_w_r, B_w_gate, B_w_up, B_w_down, gate_w,
):
    hbm = pl.BlockSpec(memory_space=pl.ANY)
    vmem = pl.BlockSpec(memory_space=pltpu.VMEM)
    out = pl.pallas_call(
        _kernel,
        out_shape=jax.ShapeDtypeStruct((S, D), BF16),
        in_specs=[hbm, hbm, hbm, hbm, vmem, hbm, hbm, hbm, vmem],
        out_specs=hbm,
        scratch_shapes=[
            pltpu.VMEM((S, D), BF16),
            pltpu.VMEM((D, 3 * D), BF16),
            pltpu.VMEM((H, DH, DH), BF16),
            pltpu.VMEM((D, D), BF16),
            pltpu.VMEM((D, F), BF16),
            pltpu.VMEM((D, F), BF16),
            pltpu.VMEM((F, D), BF16),
            pltpu.VMEM((3 * D, D), BF16),
            pltpu.VMEM((NP, AUG, 128), F32),
            pltpu.VMEM((NP, AUG, 128), BF16),
            pltpu.VMEM((D, S), BF16),
            pltpu.VMEM((S, 1), F32),
            pltpu.VMEM((D, 128), F32),
            pltpu.VMEM((F, 128), F32),
            pltpu.VMEM((S, D), BF16),
            pltpu.SemaphoreType.DMA((16,)),
            pltpu.SemaphoreType.DMA((NT_,)),
        ],
        compiler_params=pltpu.CompilerParams(vmem_limit_bytes=110 * 2**20),
    )(A_x.reshape(S, D), A_wqkv, A_w_phi, A_wo, B_w_r,
      B_w_gate, B_w_up, B_w_down, gate_w)
    return out.reshape(1, S, D)
```

```python
import math

import jax
import jax.numpy as jnp
from jax import lax
import jax.experimental.pallas as pl
import jax.experimental.pallas.tpu as pltpu

S, D, H, DH, F = 2048, 1024, 32, 32, 3584
T = 512
NTILE = S // T
NC = T // 128
NP = H // 2
AUG = 80
LOG2E = math.log2(math.e)
F32, BF16, U32 = jnp.float32, jnp.bfloat16, jnp.uint32
_NN = (((1,), (0,)), ((), ()))
_NT = (((1,), (1,)), ((), ()))
SCOPES = False
CFG = dict(
    phi_due=["v0"],
    gates=["q1.0", "q2.0", "q3.0", "kv1"],
    ohi=0.7,
    wd="q2",
    mix=(0.1, 0.9),
    side={
        "v1": [("s", 0, 8, 0.0, 1.0)],
        "k2": [("s", 8, 16, 0.05, 1.0)],
        "v2": [("r", 0, 1, 0.0, 1.0)],
        "v3": [("g", 0, 10, 0.0, 1.0)],
        "q1": [("g", 10, 20, 0.0, 1.0)],
        "q2": [("g", 20, 28, 0.0, 1.0)],
        "q3": [("d", 0, 8, 0.0, 1.0)],
    },
)

NGATE = 2 + len(CFG["gates"])


def _dot(a, b, dn):
    return lax.dot_general(a, b, dn, preferred_element_type=F32)


def _allreduce(v, op):
    v = op(v, pltpu.roll(v, 4, 0))
    return op(v, pltpu.roll(v, 2, 0))


def _phi(p):
    n = p.shape[1]
    p = p.reshape(8, 8, n)
    mx = _allreduce(jnp.max(p, axis=0), jnp.maximum)
    mn = _allreduce(jnp.min(p, axis=0), jnp.minimum)
    ep = jnp.exp2(p - mx[None])
    en = jnp.exp2(mn[None] - p)
    rp = 1.0 / _allreduce(jnp.sum(ep, axis=0), jnp.add)
    rn = 1.0 / _allreduce(jnp.sum(en, axis=0), jnp.add)
    fp = (ep * rp[None]).reshape(64, n).astype(BF16)
    fn = (en * rn[None]).reshape(64, n).astype(BF16)
    return jnp.concatenate([fp, fn], axis=0)


def _sublane_allsum(v):
    v = v + pltpu.roll(v, 4, 0)
    v = v + pltpu.roll(v, 2, 0)
    return v + pltpu.roll(v, 1, 0)


def _to_col(row8):
    return jnp.broadcast_to(row8[0:1], (128, 128)).T


def _kernel(x_hbm, wqkv_hbm, wphi_hbm, wo_hbm, wr_ref, wg_hbm, wu_hbm, wd_hbm, gw_ref,
            out_hbm,
            x_v, wqkv_v, wphi_v, wo_v, wg_v, wu_v, wd_v,
            wt_v, kv_v, kvm_v, o_v, r_v, g_v, xcol_v, hcol_v, y_v, x2_v, out_v,
            sems, osems):
    copies = {}
    out_copies = []

    def start(name, src, dst):
        c = pltpu.make_async_copy(src, dst, sems.at[len(copies)])
        copies[name] = c
        c.start()

    def wait(*names):
        for n in names:
            if SCOPES:
                with jax.named_scope("w_" + n):
                    copies[n].wait()
            else:
                copies[n].wait()

    def start_w(name, c0, c1):
        start(name, wqkv_hbm.at[:, c0:c1], wqkv_v.at[:, c0:c1])

    def start_x(name, r0, r1):
        start(name, x_hbm.at[r0:r1], x_v.at[r0:r1])

    def send(r0, r1, c0, c1):
        c = pltpu.make_async_copy(out_v.at[r0:r1, c0:c1], out_hbm.at[r0:r1, c0:c1],
                                  osems.at[len(out_copies)])
        c.start()
        out_copies.append(c)

    never = jnp.exp2(-jnp.abs(jnp.broadcast_to(
        wr_ref[...].astype(F32).reshape(1, D)[:, :128], (8, 128)))) > 2.0

    def token(v):
        v = pltpu.bitcast(v, U32)
        t = None
        for r in range(0, v.shape[0], 8):
            for c in range(0, v.shape[1], 128):
                u = v[r:r + 8, c:c + 128]
                t = u if t is None else t | u
        return t

    def spread(job, n, lo, hi):
        job = iter(job)
        return [(lo + (hi - lo) * (j + 1) / n, job) for j in range(n)]

    def matmul(lhs_ref, r0, r1, rhs, dn, due=(), then=lambda c, v: v, name=None):
        groups = (r1 - r0) // 16
        slots = len(rhs) * 2 * groups
        due = sorted(due, key=lambda e: e[0])
        res = []
        for c, b in enumerate(rhs):
            gate(f"{name}.{c}")
            at = {}
            for frac, job in due:
                s = min(int(frac * slots), slots - 1)
                if s // (2 * groups) == c:
                    t = next(job)
                    at[s] = t if s not in at else at[s] | t
            a = lhs_ref[r0 // 2:r1 // 2, :]
            parts, done = [], 0
            for m in range(groups):
                s0, s1 = 2 * c * groups + m, (2 * c + 1) * groups + m
                if s0 not in at and s1 not in at:
                    continue
                if done < m:
                    parts.append(a[8 * done:8 * m])
                blk = a[8 * m:8 * m + 8]
                lo, hi = blk[:, 0:128], blk[:, 512:640]
                if s0 in at:
                    lo = jnp.where(never, at[s0], lo)
                if s1 in at:
                    hi = jnp.where(never, at[s1], hi)
                parts.append(jnp.concatenate([lo, blk[:, 128:512], hi, blk[:, 640:]], axis=1))
                done = m + 1
            if done < groups:
                parts.append(a[8 * done:])
            a = jnp.concatenate(parts, axis=0) if len(parts) > 1 else parts[0]
            res.append(then(c, _dot(pltpu.bitcast(a, BF16), b(), dn)))
        return res

    def prep(src_col, dst_row, g0, g1):
        c = lax.broadcasted_iota(jnp.int32, (128, DH), 0)
        f = lax.broadcasted_iota(jnp.int32, (128, DH), 1)
        sel = jnp.where(((c & 63) >> 1) == f, 1.0, 0.0).astype(BF16)
        c = lax.broadcasted_iota(jnp.int32, (128, 128), 0)
        hd = lax.broadcasted_iota(jnp.int32, (128, 128), 1)
        keep = (((c >> 6) << 1) + (c & 1)) == (hd >> 5)
        ms = []
        for g in range(g0, g1):
            wblk = wphi_v[4 * g:4 * g + 4].reshape(128, DH)
            ms.append(jnp.where(keep, _dot(sel, wblk, _NT), 0.0).astype(BF16))
        for g, m in zip(range(g0, g1), ms):
            w = wqkv_v[:, src_col + 128 * g:src_col + 128 * (g + 1)]
            wt_v[dst_row // 2 + 64 * g:dst_row // 2 + 64 * (g + 1), :] = pltpu.bitcast(
                (_dot(m, w, _NT) * LOG2E).astype(BF16), U32)

    def prep_v():
        for g in range(D // 128):
            for c in range(D // 128):
                w = pltpu.bitcast(wqkv_v[128 * c:128 * (c + 1),
                                         2 * D + 128 * g:2 * D + 128 * (g + 1)].T, U32)
                wt_v[D // 2 + 64 * g:D // 2 + 64 * (g + 1), 128 * c:128 * (c + 1)] = w
                yield token(w[56:64])

    def x_chunks(c0, c1):
        return [lambda c=c: x_v[128 * c:128 * (c + 1), :] for c in range(c0, c1)]

    def x_tile(i):
        return x_chunks(NC * i, NC * (i + 1))

    def features(_, p):
        return [_phi(p[64 * j:64 * (j + 1)]) for j in range(NP)]

    def phi_due(name, phi, lo, hi):
        if name not in CFG["phi_due"]:
            return []
        return spread((token(f) for fs in phi for f in fs), NC * NP, lo, hi)

    def kv_update(i, phi, vt):
        ones = jnp.ones((AUG - 64, T), BF16)
        for p in range(NP):
            f = jnp.concatenate([fs[p] for fs in phi], axis=1)
            v = jnp.concatenate([v[64 * p:64 * (p + 1)].astype(BF16) for v in vt], axis=1)
            kv = _dot(jnp.concatenate([v, ones], axis=0), f, _NT)
            if i > 0:
                kv = kv + kv_v[p]
            if i < NTILE - 1:
                kv_v[p] = kv
            else:
                r = lax.broadcasted_iota(jnp.int32, (AUG, 128), 0)
                c = lax.broadcasted_iota(jnp.int32, (AUG, 128), 1)
                keep = jnp.where(r < 64, r >> 5, (r - 64) >> 3) == (c & 1)
                kvm_v[p] = pltpu.bitcast(jnp.where(keep, kv, 0.0).astype(BF16), U32)

    def attend(phi):
        ot = []
        for p in range(NP):
            f = jnp.concatenate([fs[p] for fs in phi], axis=1)
            nd = _dot(pltpu.bitcast(kvm_v[p], BF16), f, _NN)
            r0 = 1.0 / (nd[64:72] + 1e-6)
            r1 = 1.0 / (nd[72:80] + 1e-6)
            o0 = (nd[0:32].reshape(4, 8, T) * r0[None]).reshape(32, T)
            o1 = (nd[32:64].reshape(4, 8, T) * r1[None]).reshape(32, T)
            ot.append(jnp.concatenate([o0, o1], axis=0).astype(BF16))
        return ot

    def put_o(slot, ot):
        for q in range(NP // 2):
            two = jnp.concatenate(ot[2 * q:2 * q + 2], axis=0)
            for c in range(NC):
                o = pltpu.bitcast(two[:, 128 * c:128 * (c + 1)].T, U32)
                o_v[slot, 64 * c:64 * (c + 1), 128 * q:128 * (q + 1)] = o
                yield o[56:64]

    def scores(j0, j1):
        wr = wr_ref[...].astype(F32).reshape(1, D)
        gw = gw_ref[...].astype(F32).reshape(1, D)
        for j in range(j0, j1):
            rs, gs = [], []
            for m in range(128 * j, 128 * (j + 1), 16):
                b = x_v[m:m + 16, :].astype(F32)
                r, g = b * wr, b * gw
                for parts, v in ((rs, r), (gs, g)):
                    acc = v[:, 0:128]
                    for c in range(128, D, 128):
                        acc = acc + v[:, c:c + 128]
                    parts.append(acc)
                yield token(jnp.concatenate([rs[-1], gs[-1]], axis=0))
            r = jnp.concatenate(rs, axis=0).T.reshape(16, 8, 128).sum(axis=0)
            g = jnp.concatenate(gs, axis=0).T.reshape(16, 8, 128).sum(axis=0)
            r = _sublane_allsum(r)
            r_v[8 * j:8 * (j + 1), :] = r
            g = _to_col(jax.nn.sigmoid(_sublane_allsum(g)))
            g_v[128 * j:128 * (j + 1), :] = g
            yield token(r) | token(g[120:128])

    routed = []

    def route():
        r = r_v[...].astype(BF16).astype(F32)
        bits = lax.bitcast_convert_type(jnp.where(r == 0.0, 0.0, r), jnp.int32)
        key = jnp.where(bits < 0, bits ^ 0x7FFFFFFF, bits)
        key = jnp.where(r != r, jnp.iinfo(jnp.int32).min, key)
        pos = ((lax.broadcasted_iota(jnp.int32, r.shape, 0) >> 3) * 128
               + lax.broadcasted_iota(jnp.int32, r.shape, 1))
        idx = jnp.min(jnp.where(key == jnp.max(key), pos, S))
        base = pl.multiple_of((idx >> 4) << 4, 16)
        blk = x_v[pl.ds(base, 16), :].astype(F32)
        sub = lax.broadcasted_iota(jnp.int32, (16, D), 0)
        blk = jnp.where(sub == (idx & 15), blk, 0.0)
        row = _sublane_allsum(blk[:8] + blk[8:])
        routed.append(idx)
        for j in range(D // 128):
            col = _to_col(row[:, 128 * j:128 * (j + 1)])
            xcol_v[128 * j:128 * (j + 1), :] = col
            yield token(col[120:128])
        r_sel = jnp.sum(jnp.where(pos == idx, r, 0.0).reshape(-1, 8, 128).sum(axis=0),
                        axis=1, keepdims=True)
        y_v[...] = jnp.broadcast_to(jax.nn.sigmoid(r_sel), (8, D))
        yield token(y_v[:, 0:128])

    def matvec(w_ref, col_ref, n, j):
        acc = None
        for k in range(0, n, 16):
            w = w_ref[k:k + 16, 128 * j:128 * (j + 1)].astype(F32) * col_ref[k:k + 16, :]
            acc = (w[:8] if acc is None else acc + w[:8]) + w[8:]
            if k % 256 == 240:
                yield token(acc)
        return _sublane_allsum(acc)

    def gate_up(j0, j1):
        for j in range(j0, j1):
            g = yield from matvec(wg_v, xcol_v, D, j)
            u = yield from matvec(wu_v, xcol_v, D, j)
            h = _to_col(g * jax.nn.sigmoid(g) * u)
            hcol_v[128 * j:128 * (j + 1), :] = h
            yield token(h[120:128])

    def down(j0, j1):
        for j in range(j0, j1):
            part = yield from matvec(wd_v, hcol_v, F, j)
            y_v[:, 128 * j:128 * (j + 1)] *= part
            yield token(part)

    def side(name):
        due = []
        for kind, j0, j1, lo, hi in CFG["side"].get(name, []):
            job, steps = {"s": (scores, 9), "g": (gate_up, 9), "d": (down, 15),
                          "r": (lambda *_: route(), 9)}[kind]
            due += spread(job(j0, j1), steps * (j1 - j0), lo, hi)
        return due

    def add_routed(idx, n):
        base = pl.multiple_of(jnp.minimum((idx >> 4) << 4, n - 16), 16)
        hit = lax.broadcasted_iota(jnp.int32, (16, D), 0) + base == idx
        h = jnp.tile(1.0 - g_v[pl.ds(base, 16), :], (1, D // 128))
        cur = out_v[pl.ds(base, 16), :].astype(F32)
        out_v[pl.ds(base, 16), :] = jnp.where(hit, cur + h * y_v[0:1, :], cur).astype(BF16)

    def project(i, j0, j1, due, mixed=(), idx=None):
        rows = slice(i * T, (i + 1) * T)
        n = j1 - j0
        for j in range(j0, j1):
            cols = slice(128 * j, 128 * (j + 1))
            mine = [(f * n - (j - j0), t) for f, t in due
                    if min(int(f * n), n - 1) == j - j0]
            a, = matmul(o_v.at[i % 2], 0, T, [lambda: wo_v[:, cols]], _NN,
                        mine + spread(mixed, len(mixed), *CFG['mix']))
            g = g_v[rows, :]
            b = x_v[rows, cols].astype(F32)
            upd = b * 0.0
            if idx is not None:
                hit = lax.broadcasted_iota(jnp.int32, (T, 128), 0) + i * T == idx
                upd = upd + jnp.where(hit, y_v[0:1, cols], 0.0)
            out = (g * a + (1.0 - g) * (b + upd)).astype(BF16)
            out_v[rows, cols] = out
            mixed = [token(out[64 * m:64 * (m + 1)]) for m in range(T // 64)]
        return mixed

    gates = iter(range(NGATE))

    def gate(name=None):
        if name is None or name in CFG["gates"]:
            g = next(gates)
            wait(f"gate{g}")
            if name is not None and name.startswith(CFG["wd"]):
                wait("wd")

    start("wphi0", wphi_hbm.at[0:8], wphi_v.at[0:8])
    start_w("wk0", D, D + 256)
    start_x("x0a", 0, 256)
    start("wphi1", wphi_hbm.at[8:H], wphi_v.at[8:H])
    start_w("wk1", D + 256, D + 512)
    start_x("x0b", 256, 512)
    start_w("wk2", D + 512, 2 * D)
    start_w("wv", 2 * D, 3 * D)
    for i in range(NGATE):
        start(f"gate{i}", x_hbm.at[0:16], x2_v.at[i])
    start_x("x1", T, S)
    start_w("wq", 0, D)
    start("wg", wg_hbm, wg_v)
    start("wu", wu_hbm, wu_v)
    start("wo", wo_hbm, wo_v)
    start("wd", wd_hbm, wd_v)
    wait("wphi0", "wk0", "x0a")
    prep(D, 0, 0, 2)
    k00 = matmul(wt_v, 0, 256, x_chunks(0, 2), _NT)
    wait("wphi1", "wk1", "x0b")
    prep(D, 0, 2, 4)
    k01 = matmul(wt_v, 0, 256, x_chunks(2, 4), _NT)
    k1 = matmul(wt_v, 256, 512, x_chunks(0, 4), _NT)
    wait("wk2")
    prep(D, 0, 4, 8)
    k2 = matmul(wt_v, 512, D, x_chunks(0, 2), _NT)
    wait("wv")
    k2 += matmul(wt_v, 512, D, x_chunks(2, 4), _NT, spread(prep_v(), 64, 0.1, 1.0))
    phi = [features(0, jnp.concatenate(k, axis=0)) for k in zip(k00 + k01, k1, k2)]
    vt = matmul(wt_v, D, 2 * D, x_tile(0), _NT, phi_due("v0", phi, 0.0, 1.0) + side("v0"), name="v0")
    kv_update(0, phi, vt)

    wait("x1")
    for i in (1, 2):
        phi = matmul(wt_v, 0, D, x_tile(i), _NT, side(f"k{i}"), features, f"k{i}")
        vt = matmul(wt_v, D, 2 * D, x_tile(i), _NT, phi_due(f"v{i}", phi, 0.0, 1.0) + side(f"v{i}"), name=f"v{i}")
        kv_update(i, phi, vt)
        gate(f"kv{i}")

    wait("wq", "wg", "wu", "wo")
    phi = matmul(wt_v, 0, D, x_tile(3), _NT, side("k3"), features, "k3")
    prep(0, 2 * D, 0, D // 128)
    phiq = matmul(wt_v, 2 * D, 3 * D, x_tile(0), _NT, phi_due("q0", phi, 0.0, 1.0) + side("q0"),
                  features, "q0")
    vt = matmul(wt_v, D, 2 * D, x_tile(3), _NT, phi_due("v3", phiq, 0.0, 1.0) + side("v3"), name="v3")
    kv_update(3, phi, vt)
    odue = put_o(0, attend(phiq))

    mixed = []
    for i in range(1, NTILE):
        hi = 1.0
        for c in range(NC):
            if f"q{i}.{c}" in CFG["gates"]:
                hi = c / NC - 0.01
        if hi < 0:
            hi, mixed = CFG["ohi"], []
        phiq = matmul(wt_v, 2 * D, 3 * D, x_tile(i), _NT,
                      spread(odue, 32 if odue else 0, 0.1 * hi, hi)
                      + spread(mixed, len(mixed), 0.0, 0.1) + side(f"q{i}"), features, f"q{i}")
        if i < NTILE - 1:
            mixed = project(i - 1, 0, 8, phi_due(f"w{i - 1}", phiq, 0.0, 1.0) + side(f"w{i - 1}"))
            odue = put_o(i % 2, attend(phiq))
        else:
            mixed = project(i - 1, 0, 5, phi_due(f"w{i - 1}", phiq, 0.0, 1.0) + side(f"w{i - 1}"))
            odue = put_o(i % 2, attend(phiq))
            project(i - 1, 5, 8, spread(odue, 32, 0.2, 1.0), mixed)
    idx, = routed
    add_routed(idx, S - T)
    send(0, S - T, 0, D)
    gate()
    project(NTILE - 1, 0, 5, [], idx=idx)
    send(S - T, S, 0, 640)
    gate()
    project(NTILE - 1, 5, 8, [], idx=idx)
    send(S - T, S, 640, D)
    if SCOPES:
        with jax.named_scope("w_out"):
            for c in out_copies:
                c.wait()
    else:
        for c in out_copies:
            c.wait()


@jax.jit
def pallas_gated_mix__linear_kernel_hedgehog__moe_arch_mod__prompt_kernel(
    A_x, A_wqkv, A_w_phi, A_wo, B_x, B_w_r, B_w_gate, B_w_up, B_w_down, gate_w,
):
    del B_x
    hbm = pl.BlockSpec(memory_space=pl.ANY)
    vmem = pl.BlockSpec(memory_space=pltpu.VMEM)
    out = pl.pallas_call(
        _kernel,
        out_shape=jax.ShapeDtypeStruct((S, D), BF16),
        in_specs=[hbm, hbm, hbm, hbm, vmem, hbm, hbm, hbm, vmem],
        out_specs=hbm,
        scratch_shapes=[
            pltpu.VMEM((S, D), BF16),
            pltpu.VMEM((D, 3 * D), BF16),
            pltpu.VMEM((H, DH, DH), BF16),
            pltpu.VMEM((D, D), BF16),
            pltpu.VMEM((D, F), BF16),
            pltpu.VMEM((D, F), BF16),
            pltpu.VMEM((F, D), BF16),
            pltpu.VMEM((3 * D // 2, D), U32),
            pltpu.VMEM((NP, AUG, 128), F32),
            pltpu.VMEM((NP, AUG // 2, 128), U32),
            pltpu.VMEM((2, T // 2, D), U32),
            pltpu.VMEM((S // 16, 128), F32),
            pltpu.VMEM((S, 128), F32),
            pltpu.VMEM((D, 128), F32),
            pltpu.VMEM((F, 128), F32),
            pltpu.VMEM((8, D), F32),
            pltpu.VMEM((NGATE, 16, D), BF16),
            pltpu.VMEM((S, D), BF16),
            pltpu.SemaphoreType.DMA((16 + NGATE,)),
            pltpu.SemaphoreType.DMA((4,)),
        ],
        compiler_params=pltpu.CompilerParams(vmem_limit_bytes=110 * 2**20),
    )(A_x.reshape(S, D), A_wqkv, A_w_phi, A_wo, B_w_r,
      B_w_gate, B_w_up, B_w_down, gate_w)
    return out.reshape(1, S, D)
```

```python
import math

import jax
import jax.numpy as jnp
from jax import lax
import jax.experimental.pallas as pl
import jax.experimental.pallas.tpu as pltpu

S, D, H, DH, F = 2048, 1024, 32, 32, 3584
T = 512
NTILE = S // T
NC = T // 128
NP = H // 2
AUG = 80
LOG2E = math.log2(math.e)
F32, BF16, U32 = jnp.float32, jnp.bfloat16, jnp.uint32
_NN = (((1,), (0,)), ((), ()))
_NT = (((1,), (1,)), ((), ()))
SCOPES = False
CFG = dict(
    pv=2.0,
    mixtok=8,
    last=4,
    w2=5,
    stages=[(3, 2), (6, 2), (8, 4)],
    hold=2,
    phi=(0.0, 0.8),
    phi_due=["v0"],
    gates=["k1.0", "k2.0", "k3.0", "q1.0", "q2.0", "q3.0"],
    ohi=0.7,
    waits={"k1.0": ["x1"], "k3.0": ["wq", "wo", "wg", "wu"], "q1.0": ["wd"]},
    mix=(0.1, 0.9),
    side={
        "v1": [("s", 0, 8, 0.0, 1.0)],
        "k2": [("s", 8, 16, 0.05, 1.0)],
        "v2": [("r", 0, 1, 0.0, 1.0)],
        "v3": [("g", 0, 14, 0.0, 1.0)],
        "q1": [("g", 14, 28, 0.0, 1.0)],
        "q2": [("d", 0, 8, 0.0, 1.0)],
    },
)
CFG["side"].update(k1=[("s",12,16,0.1,1)], v1=[("s",0,8,0,1)], k2=[], v2=[("s",8,12,0,0.35),("r",0,1,0.5,1)])
NGATE = 1 + len(CFG["gates"])


def _dot(a, b, dn):
    return lax.dot_general(a, b, dn, preferred_element_type=F32)


def _allreduce(v, op):
    v = op(v, pltpu.roll(v, 4, 0))
    return op(v, pltpu.roll(v, 2, 0))


def _recip(s):
    r = pl.reciprocal(s, approx=True)
    return r * (2.0 - s * r)


def _phi(p):
    n = p.shape[1]
    p = p.reshape(8, 8, n)
    mx = _allreduce(jnp.max(p, axis=0), jnp.maximum)
    mn = _allreduce(jnp.min(p, axis=0), jnp.minimum)
    ep = jnp.exp2(p - mx[None])
    en = jnp.exp2(mn[None] - p)
    rp = _recip(_allreduce(jnp.sum(ep, axis=0), jnp.add))
    rn = _recip(_allreduce(jnp.sum(en, axis=0), jnp.add))
    f = jnp.concatenate([ep * rp[None], en * rn[None]], axis=0).reshape(128, n)
    return f, jnp.concatenate([rp, rn], axis=0)


def _sublane_allsum(v):
    v = v + pltpu.roll(v, 4, 0)
    v = v + pltpu.roll(v, 2, 0)
    return v + pltpu.roll(v, 1, 0)


def _to_col(row8):
    return jnp.broadcast_to(row8[0:1], (128, 128)).T


def _kernel(x_hbm, wqkv_hbm, wphi_hbm, wo_hbm, wr_hbm, wg_hbm, wu_hbm, wd_hbm, gw_hbm,
            out_hbm,
            wr_ref, gw_ref, x_v, wqkv_v, wphi_v, wo_v, wg_v, wu_v, wd_v,
            wk_v, wv_v, wq_v, kv_v, kvm_v, o_v, r_v, g_v, xcol_v, hcol_v, y_v, x2_v, out_v,
            sems, osems):
    copies = {}
    out_copies = []

    def start(name, src, dst):
        c = pltpu.make_async_copy(src, dst, sems.at[len(copies)])
        copies[name] = c
        c.start()

    waited = []

    def wait(*names):
        for n in names:
            waited.append(n)
            if SCOPES:
                with jax.named_scope("w_" + n):
                    copies[n].wait()
            else:
                copies[n].wait()

    def start_w(name, c0, c1):
        start(name, wqkv_hbm.at[:, c0:c1], wqkv_v.at[:, c0:c1])

    def start_x(name, r0, r1):
        start(name, x_hbm.at[r0:r1], x_v.at[r0:r1])

    def send(r0, r1, c0, c1):
        c = pltpu.make_async_copy(out_v.at[r0:r1, c0:c1], out_hbm.at[r0:r1, c0:c1],
                                  osems.at[len(out_copies)])
        c.start()
        out_copies.append(c)

    def token(v):
        v = pltpu.bitcast(v, U32)
        t = None
        for r in range(0, v.shape[0], 8):
            for c in range(0, v.shape[1], 128):
                u = v[r:r + 8, c:c + 128]
                t = u if t is None else t | u
        return t

    def spread(job, n, lo, hi):
        job = iter(job)
        return [(lo + (hi - lo) * (j + 1) / n, job) for j in range(n)]

    def matmul(lhs_ref, r0, r1, rhs, dn, due=(), then=lambda c, v: v, name=None):
        groups = (r1 - r0) // 16
        slots = len(rhs) * 2 * groups
        due = sorted(due, key=lambda e: e[0])
        res = []
        for c, b in enumerate(rhs):
            gate(f"{name}.{c}")
            at = {}
            for frac, job in due:
                s = min(int(frac * slots), slots - 1)
                if s // (2 * groups) == c and frac <= 1.0:
                    t = next(job)
                    at[s] = t if s not in at else at[s] | t
            a = lhs_ref[r0 // 2:r1 // 2, :]
            parts, done = [], 0
            for m in range(groups):
                s0, s1 = 2 * c * groups + m, (2 * c + 1) * groups + m
                if s0 not in at and s1 not in at:
                    continue
                if done < m:
                    parts.append(a[8 * done:8 * m])
                blk = a[8 * m:8 * m + 8]
                lo, hi = blk[:, 0:128], blk[:, 512:640]
                if s0 in at:
                    lo = jnp.where(never, at[s0], lo)
                if s1 in at:
                    hi = jnp.where(never, at[s1], hi)
                parts.append(jnp.concatenate([lo, blk[:, 128:512], hi, blk[:, 640:]], axis=1))
                done = m + 1
            if done < groups:
                parts.append(a[8 * done:])
            a = jnp.concatenate(parts, axis=0) if len(parts) > 1 else parts[0]
            res.append(then(c, _dot(pltpu.bitcast(a, BF16), b(), dn)))
        for frac, job in due:
            if frac > 1.0:
                next(job)
        return res

    def prep(src_col, dst, g0, g1):
        c = lax.broadcasted_iota(jnp.int32, (64, DH), 0)
        f = lax.broadcasted_iota(jnp.int32, (64, DH), 1)
        sel = jnp.where((c >> 1) == f, 1.0, 0.0).astype(BF16)
        c = lax.broadcasted_iota(jnp.int32, (128, 128), 0)
        hd = lax.broadcasted_iota(jnp.int32, (128, 128), 1)
        keep = (((c >> 6) << 1) + (c & 1)) == (hd >> 5)
        ms = []
        for g in range(g0, g1):
            wblk = wphi_v[4 * g:4 * g + 4].reshape(128, DH)
            m = _dot(sel, wblk, _NT)
            ms.append(jnp.where(keep, jnp.concatenate([m, m], axis=0), 0.0).astype(BF16))
        for g, m in zip(range(g0, g1), ms):
            w = wqkv_v[:, src_col + 128 * g:src_col + 128 * (g + 1)]
            w = pltpu.bitcast((_dot(m, w, _NT) * LOG2E).astype(BF16), U32)
            for n in range(dst.shape[0]):
                dst[n, 64 * g:64 * (g + 1), :] = w

    def prep_v():
        for g, c in ((g, c) for h in (0, 4) for g in range(8) for c in range(h, h + 4)):
            if True:
                w = pltpu.bitcast(wqkv_v[128 * c:128 * (c + 1),
                                         2 * D + 128 * g:2 * D + 128 * (g + 1)].T, U32)
                for n in range(wv_v.shape[0]):
                    wv_v[n, 64 * g:64 * (g + 1), 128 * c:128 * (c + 1)] = w
                yield token(w[56:64])

    def x_chunks(c0, c1):
        return [lambda c=c: x_v[128 * c:128 * (c + 1), :] for c in range(c0, c1)]

    def x_tile(i):
        return x_chunks(NC * i, NC * (i + 1))

    def features(c, p, tile):
        row = []
        for j in range(NP):
            f, r = _phi(p[64 * j:64 * (j + 1)])
            row.append((f.astype(BF16), r))
        return row

    def phi_due(name, ps):
        if name not in CFG["phi_due"]:
            return []
        return spread((token(r) for row in ps for _, r in row), NC * NP, *CFG["phi"])

    def wide(ps, j):
        return jnp.concatenate([row[j][0] for row in ps], axis=1)

    odd = lax.broadcasted_iota(jnp.int32, (1, 128), 1) & 1

    def kv_update(i, phi, vt):
        m = AUG
        for p in range(NP):
            v = jnp.concatenate([v[64 * p:64 * (p + 1)].astype(BF16) for v in vt], axis=1)
            if m > 64:
                v = jnp.concatenate([v, jnp.ones((m - 64, T), BF16)], axis=0)
            kv = _dot(v, wide(phi, p), _NT)
            if i > 0:
                kv = kv + kv_v[p, 0:m]
            if i < NTILE - 1:
                kv_v[p, 0:m] = kv
            else:
                r = lax.broadcasted_iota(jnp.int32, (m, 128), 0)
                keep = jnp.where(r < 64, r >> 5, (r - 64) >> 3) == odd
                kvm_v[p, 0:m // 2] = pltpu.bitcast(jnp.where(keep, kv, 0.0).astype(BF16), U32)

    def attend(phi):
        ot = []
        for p in range(NP):
            f = wide(phi, p)
            nd = _dot(pltpu.bitcast(kvm_v[p], BF16), f, _NN)
            r0 = _recip(nd[64:72] + 1e-6)
            r1 = _recip(nd[72:80] + 1e-6)
            o0 = (nd[0:32].reshape(4, 8, T) * r0[None]).reshape(32, T)
            o1 = (nd[32:64].reshape(4, 8, T) * r1[None]).reshape(32, T)
            ot.append(jnp.concatenate([o0, o1], axis=0).astype(BF16))
        return ot

    def put_o(slot, ot):
        for q in range(NP // 2):
            two = jnp.concatenate(ot[2 * q:2 * q + 2], axis=0)
            for c in range(NC):
                o = pltpu.bitcast(two[:, 128 * c:128 * (c + 1)].T, U32)
                o_v[slot, 64 * c:64 * (c + 1), 128 * q:128 * (q + 1)] = o
                yield o[56:64]

    def scores(j0, j1):
        wr = wr_ref[...].astype(F32).reshape(1, D)
        gw = gw_ref[...].astype(F32).reshape(1, D)
        for j in range(j0, j1):
            rs, gs = [], []
            for m in range(128 * j, 128 * (j + 1), 16):
                b = x_v[m:m + 16, :].astype(F32)
                r, g = b * wr, b * gw
                for parts, v in ((rs, r), (gs, g)):
                    acc = v[:, 0:128]
                    for c in range(128, D, 128):
                        acc = acc + v[:, c:c + 128]
                    parts.append(acc)
                yield token(jnp.concatenate([rs[-1], gs[-1]], axis=0))
            r = jnp.concatenate(rs, axis=0).T.reshape(16, 8, 128).sum(axis=0)
            g = jnp.concatenate(gs, axis=0).T.reshape(16, 8, 128).sum(axis=0)
            r = _sublane_allsum(r)
            r_v[8 * j:8 * (j + 1), :] = r
            g = _to_col(jax.nn.sigmoid(_sublane_allsum(g)))
            g_v[128 * j:128 * (j + 1), :] = g
            yield token(r) | token(g[120:128])

    routed = []

    def route():
        r = r_v[...].astype(BF16).astype(F32)
        bits = lax.bitcast_convert_type(jnp.where(r == 0.0, 0.0, r), jnp.int32)
        key = jnp.where(bits < 0, bits ^ 0x7FFFFFFF, bits)
        key = jnp.where(r != r, jnp.iinfo(jnp.int32).min, key)
        pos = ((lax.broadcasted_iota(jnp.int32, r.shape, 0) >> 3) * 128
               + lax.broadcasted_iota(jnp.int32, r.shape, 1))
        idx = jnp.min(jnp.where(key == jnp.max(key), pos, S))
        base = pl.multiple_of((idx >> 4) << 4, 16)
        blk = x_v[pl.ds(base, 16), :].astype(F32)
        sub = lax.broadcasted_iota(jnp.int32, (16, D), 0)
        blk = jnp.where(sub == (idx & 15), blk, 0.0)
        row = _sublane_allsum(blk[:8] + blk[8:])
        routed.append(idx)
        for j in range(D // 128):
            col = _to_col(row[:, 128 * j:128 * (j + 1)])
            xcol_v[128 * j:128 * (j + 1), :] = col
            yield token(col[120:128])
        r_sel = jnp.sum(jnp.where(pos == idx, r, 0.0).reshape(-1, 8, 128).sum(axis=0),
                        axis=1, keepdims=True)
        y_v[...] = jnp.broadcast_to(jax.nn.sigmoid(r_sel), (8, D))
        yield token(y_v[:, 0:128])

    def matvec(w_ref, col_ref, n, j):
        acc = None
        for k in range(0, n, 16):
            w = w_ref[k:k + 16, 128 * j:128 * (j + 1)].astype(F32) * col_ref[k:k + 16, :]
            acc = (w[:8] if acc is None else acc + w[:8]) + w[8:]
            if k % 256 == 240:
                yield token(acc)
        return _sublane_allsum(acc)

    def gate_up(j0, j1):
        for j in range(j0, j1):
            g = yield from matvec(wg_v, xcol_v, D, j)
            u = yield from matvec(wu_v, xcol_v, D, j)
            h = _to_col(g * jax.nn.sigmoid(g) * u)
            hcol_v[128 * j:128 * (j + 1), :] = h
            yield token(h[120:128])

    def down(j0, j1):
        for j in range(j0, j1):
            part = yield from matvec(wd_v, hcol_v, F, j)
            y_v[:, 128 * j:128 * (j + 1)] *= part
            yield token(part)

    def side(name):
        due = []
        for kind, j0, j1, lo, hi in CFG["side"].get(name, []):
            job, steps = {"s": (scores, 9), "g": (gate_up, 9), "d": (down, 15),
                          "r": (lambda *_: route(), 9)}[kind]
            due += spread(job(j0, j1), steps * (j1 - j0), lo, hi)
        return due

    def add_routed(idx, r0, r1):
        base = pl.multiple_of(jnp.clip((idx >> 4) << 4, r0, r1 - 16), 16)
        hit = lax.broadcasted_iota(jnp.int32, (16, D), 0) + base == idx
        h = jnp.tile(1.0 - g_v[pl.ds(base, 16), :], (1, D // 128))
        cur = out_v[pl.ds(base, 16), :].astype(F32)
        out_v[pl.ds(base, 16), :] = jnp.where(hit, cur + h * y_v[0:1, :], cur).astype(BF16)

    def project(i, j0, j1, due, mixed=(), idx=None):
        rows = slice(i * T, (i + 1) * T)
        n = j1 - j0
        for j in range(j0, j1):
            cols = slice(128 * j, 128 * (j + 1))
            mine = [(f * n - (j - j0), t) for f, t in due
                    if min(int(f * n), n - 1) == j - j0]
            a, = matmul(o_v.at[i % 2], 0, T, [lambda: wo_v[:, cols]], _NN,
                        mine + spread(mixed, len(mixed), *CFG['mix']))
            g = g_v[rows, :]
            b = x_v[rows, cols].astype(F32)
            upd = b * 0.0
            if idx is not None:
                hit = lax.broadcasted_iota(jnp.int32, (T, 128), 0) + i * T == idx
                upd = upd + jnp.where(hit, y_v[0:1, cols], 0.0)
            out = g * a + (1.0 - g) * (b + upd)
            out_v[rows, cols] = out.astype(BF16)
            n_tok = CFG["mixtok"]
            mixed = [token(out[m - 8:m]) for m in range(T // n_tok, T + 1, T // n_tok)]
        return mixed

    gates = iter(range(NGATE))

    def gate(name=None):
        if name is None or name in CFG["gates"]:
            g = next(gates)
            wait(f"gate{g}")
            wait(*CFG["waits"].get(name, []))

    stages = CFG["stages"]
    g0 = c0 = 0
    need = []
    for n, (g1, c1) in enumerate(stages):
        need.append([])
        if g1 > g0:
            start_w(f"wk{n}", D + 128 * g0, D + 128 * g1)
            need[n].append(f"wk{n}")
            if n == 0:
                start("wphi0", wphi_hbm.at[0:4 * g1], wphi_v.at[0:4 * g1])
                need[n].append("wphi0")
            elif "wphi1" not in copies:
                start("wphi1", wphi_hbm.at[4 * g0:H], wphi_v.at[4 * g0:H])
                need[n].append("wphi1")
        if c1 > c0:
            start_x(f"x0{n}", 128 * c0, 128 * c1)
            need[n].append(f"x0{n}")
        g0, c0 = g1, c1
    start("wr", wr_hbm, wr_ref)
    start("gw", gw_hbm, gw_ref)
    start_w("wv", 2 * D, 3 * D)
    for i in range(NGATE):
        start(f"gate{i}", x_hbm.at[0:16], x2_v.at[i])
    start_x("x1", T, S)
    start_w("wq", 0, D)
    start("wo", wo_hbm, wo_v)
    start("wg", wg_hbm, wg_v)
    start("wu", wu_hbm, wu_v)
    start("wd", wd_hbm, wd_v)

    wk = wk_v.at[0]
    kt = [[] for _ in range(NC)]

    def keys(g0, g1, c0, c1, due=()):
        if g1 > g0 and c1 > c0:
            for c, k in enumerate(matmul(wk, 128 * g0, 128 * g1, x_chunks(c0, c1), _NT, due)):
                kt[c0 + c].append(k)

    g0 = c0 = 0
    for n, (g1, c1) in enumerate(stages):
        wait(*need[n])
        keys(0, g0, c0, c1)
        prep(D, wk_v, g0, g1)
        keys(g0, g1, 0, c1 if n + 1 < len(stages) else CFG["hold"])
        g_last, g0, c0 = g0, g1, c1
    wait("wr", "gw", "wv")
    never = jnp.exp2(-jnp.abs(jnp.broadcast_to(
        wr_ref[...].astype(F32).reshape(1, D)[:, :128], (8, 128)))) > 2.0
    keys(g_last, g0, CFG["hold"], NC, spread(prep_v(), 64, 0.1, CFG["pv"]))
    kt = [jnp.concatenate(k, axis=0) for k in kt]
    phi = [features(c, k, 0) for c, k in enumerate(kt)]
    for i in range(NTILE - 1):
        if i > 0:
            phi = matmul(wk, 0, D, x_tile(i), _NT, side(f"k{i}"), lambda c, p: features(c, p, i), f"k{i}")
        vt = matmul(wv_v.at[0], 0, D, x_tile(i), _NT,
                    phi_due(f"v{i}", phi) + side(f"v{i}"), name=f"v{i}")
        kv_update(i, phi, vt)

    phi = matmul(wk, 0, D, x_tile(3), _NT, side("k3"), lambda c, p: features(c, p, 3), "k3")
    prep(0, wq_v, 0, D // 128)
    phiq = matmul(wq_v.at[0], 0, D, x_tile(0), _NT, phi_due("q0", phi) + side("q0"),
                  lambda c, p: features(c, p, None), "q0")
    vt = matmul(wv_v.at[0], 0, D, x_tile(3), _NT, phi_due("v3", phiq) + side("v3"),
                name="v3")
    kv_update(3, phi, vt)
    odue = put_o(0, attend(phiq))

    mixed = []
    idx, = routed
    for i in range(1, NTILE):
        if i == NTILE - 1:
            add_routed(idx, 0, (i - 1) * T)
            send(0, (i - 1) * T, 0, D)
        hi = 1.0
        for c in range(NC):
            if f"q{i}.{c}" in CFG["gates"]:
                hi = c / NC - 0.01
        if hi < 0:
            hi, mixed = CFG["ohi"], []
        phiq = matmul(wq_v.at[0], 0, D, x_tile(i), _NT,
                      spread(odue, 32 if odue else 0, 0.1 * hi, hi)
                      + spread(mixed, len(mixed), 0.0, 0.1) + side(f"q{i}"), lambda c, p: features(c, p, None), f"q{i}")
        if i < NTILE - 1:
            mixed = project(i - 1, 0, 8, phi_due(f"w{i - 1}", phiq) + side(f"w{i - 1}"))
            odue = put_o(i % 2, attend(phiq))
        else:
            mixed = project(i - 1, 0, CFG['w2'], phi_due(f"w{i - 1}", phiq) + side(f"w{i - 1}"))
            odue = put_o(i % 2, attend(phiq))
            mixed = project(i - 1, CFG['w2'], 8, spread(odue, 32, 0.2, 1.0), mixed)
    n = CFG["last"]
    project(NTILE - 1, 0, n, [], mixed, idx)
    add_routed(idx, S - 2 * T, S - T)
    send(S - 2 * T, S - T, 0, D)
    send(S - T, S, 0, 128 * n)
    gate()
    project(NTILE - 1, n, 8, [], idx=idx)
    send(S - T, S, 128 * n, D)
    assert sorted(waited) == sorted(copies)
    if SCOPES:
        with jax.named_scope("w_out"):
            for c in out_copies:
                c.wait()
    else:
        for c in out_copies:
            c.wait()


@jax.jit
def pallas_gated_mix__linear_kernel_hedgehog__moe_arch_mod__prompt_kernel(
    A_x, A_wqkv, A_w_phi, A_wo, B_x, B_w_r, B_w_gate, B_w_up, B_w_down, gate_w,
):
    del B_x
    hbm = pl.BlockSpec(memory_space=pl.ANY)
    out = pl.pallas_call(
        _kernel,
        out_shape=jax.ShapeDtypeStruct((S, D), BF16),
        in_specs=[hbm] * 9,
        out_specs=hbm,
        scratch_shapes=[
            pltpu.VMEM((D,), BF16),
            pltpu.VMEM((D,), BF16),
            pltpu.VMEM((S, D), BF16),
            pltpu.VMEM((D, 3 * D), BF16),
            pltpu.VMEM((H, DH, DH), BF16),
            pltpu.VMEM((D, D), BF16),
            pltpu.VMEM((D, F), BF16),
            pltpu.VMEM((D, F), BF16),
            pltpu.VMEM((F, D), BF16),
            pltpu.VMEM((1, D // 2, D), U32),
            pltpu.VMEM((1, D // 2, D), U32),
            pltpu.VMEM((1, D // 2, D), U32),
            pltpu.VMEM((NP, AUG, 128), F32),
            pltpu.VMEM((NP, AUG // 2, 128), U32),
            pltpu.VMEM((2, T // 2, D), U32),
            pltpu.VMEM((S // 16, 128), F32),
            pltpu.VMEM((S, 128), F32),
            pltpu.VMEM((D, 128), F32),
            pltpu.VMEM((F, 128), F32),
            pltpu.VMEM((8, D), F32),
            pltpu.VMEM((NGATE, 16, D), BF16),
            pltpu.VMEM((S, D), BF16),
            pltpu.SemaphoreType.DMA((24 + NGATE,)),
            pltpu.SemaphoreType.DMA((4,)),
        ],
        compiler_params=pltpu.CompilerParams(vmem_limit_bytes=110 * 2**20),
    )(A_x.reshape(S, D), A_wqkv, A_w_phi, A_wo, B_w_r,
      B_w_gate, B_w_up, B_w_down, gate_w)
    return out.reshape(1, S, D)
```

```python
import math

import jax
import jax.numpy as jnp
from jax import lax
import jax.experimental.pallas as pl
import jax.experimental.pallas.tpu as pltpu

S, D, H, DH, F = 2048, 1024, 32, 32, 3584
T = 512
NTILE = S // T
NC = T // 128
NP = H // 2
AUG = 80
NGATE = 7
STAGES = ((2, 1), (3, 2), (6, 2), (8, 4))
LOG2E = math.log2(math.e)
F32, BF16, U32 = jnp.float32, jnp.bfloat16, jnp.uint32
_NN = (((1,), (0,)), ((), ()))
_NT = (((1,), (1,)), ((), ()))


def _dot(a, b, dn):
    return lax.dot_general(a, b, dn, preferred_element_type=F32)


def _allreduce(v, op):
    v = op(v, pltpu.roll(v, 4, 0))
    return op(v, pltpu.roll(v, 2, 0))


def _recip(s):
    r = pl.reciprocal(s, approx=True)
    return r * (2.0 - s * r)


def _phi(p):
    n = p.shape[1]
    p = p.reshape(8, 8, n)
    mx = _allreduce(jnp.max(p, axis=0), jnp.maximum)
    mn = _allreduce(jnp.min(p, axis=0), jnp.minimum)
    ep = jnp.exp2(p - mx[None])
    en = jnp.exp2(mn[None] - p)
    rp = _recip(_allreduce(jnp.sum(ep, axis=0), jnp.add))
    rn = _recip(_allreduce(jnp.sum(en, axis=0), jnp.add))
    f = jnp.concatenate([ep * rp[None], en * rn[None]], axis=0).reshape(128, n)
    return f, jnp.concatenate([rp, rn], axis=0)


def _sublane_allsum(v):
    v = v + pltpu.roll(v, 4, 0)
    v = v + pltpu.roll(v, 2, 0)
    return v + pltpu.roll(v, 1, 0)


def _to_col(row8):
    return jnp.broadcast_to(row8[0:1], (128, 128)).T


def _token(v):
    v = pltpu.bitcast(v, U32)
    t = None
    for r in range(0, v.shape[0], 8):
        for c in range(0, v.shape[1], 128):
            u = v[r:r + 8, c:c + 128]
            t = u if t is None else t | u
    return t


def _spread(job, n, lo, hi):
    job = iter(job)
    return [(lo + (hi - lo) * (j + 1) / n, job) for j in range(n)]


def _kernel(x_hbm, wqkv_hbm, wphi_hbm, wo_hbm, wr_hbm, wg_hbm, wu_hbm, wd_hbm, gw_hbm,
            out_hbm,
            wr_v, gw_v, x_v, wqkv_v, wphi_v, wo_v, wg_v, wu_v, wd_v,
            wk_v, wv_v, wq_v, kv_v, kvm_v, o_v, r_v, g_v, xcol_v, hcol_v, y_v, gate_v, out_v,
            sems, osems):
    copies = {}
    out_copies = []
    waited = []

    def start(name, src, dst):
        c = pltpu.make_async_copy(src, dst, sems.at[len(copies)])
        copies[name] = c
        c.start()

    def wait(*names):
        for n in names:
            waited.append(n)
            copies[n].wait()

    def start_w(name, c0, c1):
        start(name, wqkv_hbm.at[:, c0:c1], wqkv_v.at[:, c0:c1])

    def start_x(name, r0, r1):
        start(name, x_hbm.at[r0:r1], x_v.at[r0:r1])

    def send(r0, r1, c0, c1):
        c = pltpu.make_async_copy(out_v.at[r0:r1, c0:c1], out_hbm.at[r0:r1, c0:c1],
                                  osems.at[len(out_copies)])
        c.start()
        out_copies.append(c)

    gates = iter(range(NGATE))

    def gate(*names):
        wait(f"gate{next(gates)}", *names)

    def matmul(lhs_ref, r0, r1, rhs, dn, due=(), then=lambda v: v):
        groups = (r1 - r0) // 16
        slots = len(rhs) * 2 * groups
        due = sorted(due, key=lambda e: e[0])
        res = []
        for c, b in enumerate(rhs):
            at = {}
            for frac, job in due:
                s = min(int(frac * slots), slots - 1)
                if s // (2 * groups) == c and frac <= 1.0:
                    t = next(job)
                    at[s] = t if s not in at else at[s] | t
            a = lhs_ref[r0 // 2:r1 // 2, :]
            parts, done = [], 0
            for m in range(groups):
                s0, s1 = 2 * c * groups + m, (2 * c + 1) * groups + m
                if s0 not in at and s1 not in at:
                    continue
                if done < m:
                    parts.append(a[8 * done:8 * m])
                blk = a[8 * m:8 * m + 8]
                lo, hi = blk[:, 0:128], blk[:, 512:640]
                if s0 in at:
                    lo = jnp.where(never, at[s0], lo)
                if s1 in at:
                    hi = jnp.where(never, at[s1], hi)
                parts.append(jnp.concatenate([lo, blk[:, 128:512], hi, blk[:, 640:]], axis=1))
                done = m + 1
            if done < groups:
                parts.append(a[8 * done:])
            a = jnp.concatenate(parts, axis=0) if len(parts) > 1 else parts[0]
            res.append(then(_dot(pltpu.bitcast(a, BF16), b(), dn)))
        for frac, job in due:
            if frac > 1.0:
                next(job)
        return res

    def prep(src_col, dst, g0, g1):
        c = lax.broadcasted_iota(jnp.int32, (64, DH), 0)
        f = lax.broadcasted_iota(jnp.int32, (64, DH), 1)
        sel = jnp.where((c >> 1) == f, 1.0, 0.0).astype(BF16)
        c = lax.broadcasted_iota(jnp.int32, (128, 128), 0)
        hd = lax.broadcasted_iota(jnp.int32, (128, 128), 1)
        keep = (((c >> 6) << 1) + (c & 1)) == (hd >> 5)
        ms = []
        for g in range(g0, g1):
            m = _dot(sel, wphi_v[4 * g:4 * g + 4].reshape(128, DH), _NT)
            ms.append(jnp.where(keep, jnp.concatenate([m, m], axis=0), 0.0).astype(BF16))
        for g, m in zip(range(g0, g1), ms):
            w = wqkv_v[:, src_col + 128 * g:src_col + 128 * (g + 1)]
            dst[64 * g:64 * (g + 1), :] = pltpu.bitcast(
                (_dot(m, w, _NT) * LOG2E).astype(BF16), U32)

    def prep_v():
        for g, c in ((g, c) for h in (0, 4) for g in range(8) for c in range(h, h + 4)):
            w = pltpu.bitcast(wqkv_v[128 * c:128 * (c + 1),
                                     2 * D + 128 * g:2 * D + 128 * (g + 1)].T, U32)
            wv_v[64 * g:64 * (g + 1), 128 * c:128 * (c + 1)] = w
            yield w[56:64]

    def x_chunks(c0, c1):
        return [lambda c=c: x_v[128 * c:128 * (c + 1), :] for c in range(c0, c1)]

    def x_tile(i):
        return x_chunks(NC * i, NC * (i + 1))

    def features(p):
        row = []
        for j in range(NP):
            f, r = _phi(p[64 * j:64 * (j + 1)])
            row.append((f.astype(BF16), r))
        return row

    def wide(phi, j):
        return jnp.concatenate([row[j][0] for row in phi], axis=1)

    odd = lax.broadcasted_iota(jnp.int32, (1, 128), 1) & 1

    def kv_update(i, phi, vt):
        for p in range(NP):
            v = jnp.concatenate([v[64 * p:64 * (p + 1)].astype(BF16) for v in vt], axis=1)
            v = jnp.concatenate([v, jnp.ones((AUG - 64, T), BF16)], axis=0)
            kv = _dot(v, wide(phi, p), _NT)
            if i > 0:
                kv = kv + kv_v[p]
            if i < NTILE - 1:
                kv_v[p] = kv
            else:
                r = lax.broadcasted_iota(jnp.int32, (AUG, 128), 0)
                keep = jnp.where(r < 64, r >> 5, (r - 64) >> 3) == odd
                kvm_v[p] = pltpu.bitcast(jnp.where(keep, kv, 0.0).astype(BF16), U32)

    def attend(phi):
        ot = []
        for p in range(NP):
            nd = _dot(pltpu.bitcast(kvm_v[p], BF16), wide(phi, p), _NN)
            r0 = _recip(nd[64:72] + 1e-6)
            r1 = _recip(nd[72:80] + 1e-6)
            o0 = (nd[0:32].reshape(4, 8, T) * r0[None]).reshape(32, T)
            o1 = (nd[32:64].reshape(4, 8, T) * r1[None]).reshape(32, T)
            ot.append(jnp.concatenate([o0, o1], axis=0).astype(BF16))
        return ot

    def put_o(slot, ot):
        for q in range(NP // 2):
            two = jnp.concatenate(ot[2 * q:2 * q + 2], axis=0)
            for c in range(NC):
                o = pltpu.bitcast(two[:, 128 * c:128 * (c + 1)].T, U32)
                o_v[slot, 64 * c:64 * (c + 1), 128 * q:128 * (q + 1)] = o
                yield o[56:64]

    def scores(j0, j1):
        wr = wr_v[...].astype(F32).reshape(1, D)
        gw = gw_v[...].astype(F32).reshape(1, D)
        for j in range(j0, j1):
            rs, gs = [], []
            for m in range(128 * j, 128 * (j + 1), 16):
                b = x_v[m:m + 16, :].astype(F32)
                r, g = b * wr, b * gw
                for parts, v in ((rs, r), (gs, g)):
                    acc = v[:, 0:128]
                    for c in range(128, D, 128):
                        acc = acc + v[:, c:c + 128]
                    parts.append(acc)
                yield _token(jnp.concatenate([rs[-1], gs[-1]], axis=0))
            r = jnp.concatenate(rs, axis=0).T.reshape(16, 8, 128).sum(axis=0)
            g = jnp.concatenate(gs, axis=0).T.reshape(16, 8, 128).sum(axis=0)
            r = _sublane_allsum(r)
            r_v[8 * j:8 * (j + 1), :] = r
            g = _to_col(jax.nn.sigmoid(_sublane_allsum(g)))
            g_v[128 * j:128 * (j + 1), :] = g
            yield _token(r) | _token(g[120:128])

    routed = []

    def route():
        r = r_v[...].astype(BF16).astype(F32)
        bits = lax.bitcast_convert_type(jnp.where(r == 0.0, 0.0, r), jnp.int32)
        key = jnp.where(bits < 0, bits ^ 0x7FFFFFFF, bits)
        key = jnp.where(r != r, jnp.iinfo(jnp.int32).min, key)
        pos = ((lax.broadcasted_iota(jnp.int32, r.shape, 0) >> 3) * 128
               + lax.broadcasted_iota(jnp.int32, r.shape, 1))
        top = jnp.max(jnp.max(key, axis=0, keepdims=True), axis=1, keepdims=True)
        first = jnp.where(key == top, pos, S - 1)
        first = jnp.min(jnp.min(first, axis=0, keepdims=True), axis=1, keepdims=True)
        r_sel = jnp.sum(jnp.where(pos == first, r, 0.0).reshape(-1, 8, 128).sum(axis=0),
                        axis=1, keepdims=True)
        y_v[...] = jnp.broadcast_to(r_sel, (8, D))
        yield _token(y_v[:, 0:128])
        idx = first[0, 0]
        base = pl.multiple_of((idx >> 4) << 4, 16)
        blk = x_v[pl.ds(base, 16), :].astype(F32)
        sub = lax.broadcasted_iota(jnp.int32, (16, D), 0)
        blk = jnp.where(sub == (idx & 15), blk, 0.0)
        row = _sublane_allsum(blk[:8] + blk[8:])
        routed.append(idx)
        for j in range(D // 128):
            col = _to_col(row[:, 128 * j:128 * (j + 1)])
            xcol_v[128 * j:128 * (j + 1), :] = col
            yield _token(col[120:128])

    def matvec(w_ref, col_ref, n, j):
        acc = None
        for k in range(0, n, 16):
            w = w_ref[k:k + 16, 128 * j:128 * (j + 1)].astype(F32) * col_ref[k:k + 16, :]
            acc = (w[:8] if acc is None else acc + w[:8]) + w[8:]
            if k % 256 == 240:
                yield _token(acc)
        return _sublane_allsum(acc)

    def gate_up(j0, j1):
        for j in range(j0, j1):
            g = yield from matvec(wg_v, xcol_v, D, j)
            u = yield from matvec(wu_v, xcol_v, D, j)
            h = _to_col(g * jax.nn.sigmoid(g) * u)
            hcol_v[128 * j:128 * (j + 1), :] = h
            yield _token(h[120:128])

    def down(j0, j1):
        for j in range(j0, j1):
            part = yield from matvec(wd_v, hcol_v, F, j)
            part = part * jax.nn.sigmoid(y_v[:, 128 * j:128 * (j + 1)])
            y_v[:, 128 * j:128 * (j + 1)] = part
            yield _token(part)

    def side(job, j0, j1, lo, hi):
        return _spread(job(j0, j1), (15 if job is down else 9) * (j1 - j0), lo, hi)

    def add_routed(idx, r0, r1):
        base = pl.multiple_of(jnp.clip((idx >> 4) << 4, r0, r1 - 16), 16)
        hit = lax.broadcasted_iota(jnp.int32, (16, D), 0) + base == idx
        h = jnp.tile(1.0 - g_v[pl.ds(base, 16), :], (1, D // 128))
        cur = out_v[pl.ds(base, 16), :].astype(F32)
        out_v[pl.ds(base, 16), :] = jnp.where(hit, cur + h * y_v[0:1, :], cur).astype(BF16)

    def project(i, j0, j1, due=(), mixed=(), idx=None):
        rows = slice(i * T, (i + 1) * T)
        n = j1 - j0
        for j in range(j0, j1):
            cols = slice(128 * j, 128 * (j + 1))
            mine = [(f * n - (j - j0), t) for f, t in due if min(int(f * n), n - 1) == j - j0]
            a, = matmul(o_v.at[i % 2], 0, T, [lambda: wo_v[:, cols]], _NN,
                        mine + _spread(mixed, len(mixed), 0.1, 0.9))
            g = g_v[rows, :]
            b = x_v[rows, cols].astype(F32)
            upd = b * 0.0
            if idx is not None:
                hit = lax.broadcasted_iota(jnp.int32, (T, 128), 0) + i * T == idx
                upd = upd + jnp.where(hit, y_v[0:1, cols], 0.0)
            out = g * a + (1.0 - g) * (b + upd)
            out_v[rows, cols] = out.astype(BF16)
            mixed = [_token(out[m - 8:m]) for m in (T // 2, T)]
        return mixed

    g0 = c0 = 0
    need = []
    for n, (g1, c1) in enumerate(STAGES):
        start_w(f"wk{n}", D + 128 * g0, D + 128 * g1)
        need.append([f"wk{n}"])
        if n < 2:
            heads = slice(4 * g0, 4 * g1 if n == 0 else H)
            start(f"wphi{n}", wphi_hbm.at[heads], wphi_v.at[heads])
            need[n].append(f"wphi{n}")
        if c1 > c0:
            start_x(f"x0{n}", 128 * c0, 128 * c1)
            need[n].append(f"x0{n}")
        g0, c0 = g1, c1
    start("wr", wr_hbm, wr_v)
    start("gw", gw_hbm, gw_v)
    start_w("wv", 2 * D, 3 * D)
    for i in range(NGATE):
        start(f"gate{i}", x_hbm.at[0:16], gate_v.at[i])
    start_x("x1", T, S)
    start_w("wq", 0, D)
    start("wo", wo_hbm, wo_v)
    start("wg", wg_hbm, wg_v)
    start("wu", wu_hbm, wu_v)
    start("wd", wd_hbm, wd_v)

    kt = [[] for _ in range(NC)]

    def keys(g0, g1, c0, c1, due=()):
        if g1 > g0 and c1 > c0:
            for c, k in enumerate(matmul(wk_v, 128 * g0, 128 * g1, x_chunks(c0, c1), _NT, due)):
                kt[c0 + c].append(k)

    g0 = c0 = 0
    for n, (g1, c1) in enumerate(STAGES):
        wait(*need[n])
        keys(0, g0, c0, c1)
        prep(D, wk_v, g0, g1)
        keys(g0, g1, 0, c1 if n + 1 < len(STAGES) else 2)
        g0, c0 = g1, c1
    wait("wr", "gw", "wv")
    never = jnp.exp2(-jnp.abs(jnp.broadcast_to(
        wr_v[...].astype(F32).reshape(1, D)[:, :128], (8, 128)))) > 2.0
    keys(STAGES[-2][0], g0, 2, NC, _spread(prep_v(), 64, 0.1, 1.5))

    phi = [features(jnp.concatenate(k, axis=0)) for k in kt]
    due = _spread((_token(r) for row in phi for _, r in row), NC * NP, 0.0, 0.75)
    kv_update(0, phi, matmul(wv_v, 0, D, x_tile(0), _NT, due))

    gate("x1")
    phi = matmul(wk_v, 0, D, x_tile(1), _NT, side(scores, 11, 16, 0.1, 1.0), features)
    kv_update(1, phi, matmul(wv_v, 0, D, x_tile(1), _NT, side(scores, 0, 8, 0.0, 1.0)))

    gate()
    phi = matmul(wk_v, 0, D, x_tile(2), _NT, (), features)
    due = side(scores, 8, 11, 0.0, 0.45) + _spread(route(), 9, 0.6, 1.0)
    kv_update(2, phi, matmul(wv_v, 0, D, x_tile(2), _NT, due))
    idx, = routed

    gate("wq", "wo", "wg", "wu")
    phi = matmul(wk_v, 0, D, x_tile(3), _NT, (), features)
    prep(0, wq_v, 0, D // 128)
    phiq = matmul(wq_v, 0, D, x_tile(0), _NT, (), features)
    kv_update(3, phi, matmul(wv_v, 0, D, x_tile(3), _NT, side(gate_up, 0, 13, 0.0, 1.0)))

    o = put_o(0, attend(phiq))
    gate("wd")
    due = _spread(o, 32, 0.08, 0.8) + side(gate_up, 13, 28, 0.1, 1.0)
    phiq = matmul(wq_v, 0, D, x_tile(1), _NT, due, features)
    project(0, 0, 8)

    o = put_o(1, attend(phiq))
    gate()
    due = _spread(o, 32, 0.08, 0.8) + side(down, 0, 8, 0.05, 0.9)
    phiq = matmul(wq_v, 0, D, x_tile(2), _NT, due, features)
    project(1, 0, 8)

    o = put_o(0, attend(phiq))
    add_routed(idx, 0, 2 * T)
    send(0, 2 * T, 0, D)
    gate()
    phiq = matmul(wq_v, 0, D, x_tile(3), _NT, _spread(o, 32, 0.08, 0.8), features)
    mixed = project(2, 0, 5)
    o = put_o(1, attend(phiq))
    mixed = project(2, 5, 8, _spread(o, 32, 0.2, 1.0), mixed)
    project(3, 0, 4, (), mixed, idx)
    add_routed(idx, 2 * T, 3 * T)
    send(2 * T, 3 * T, 0, D)
    send(3 * T, S, 0, 512)
    gate()
    project(3, 4, 8, idx=idx)
    send(3 * T, S, 512, D)
    assert sorted(waited) == sorted(copies)
    for c in out_copies:
        c.wait()


@jax.jit
def pallas_gated_mix__linear_kernel_hedgehog__moe_arch_mod__prompt_kernel(
    A_x: jax.Array,
    A_wqkv: jax.Array,
    A_w_phi: jax.Array,
    A_wo: jax.Array,
    B_x: jax.Array,
    B_w_r: jax.Array,
    B_w_gate: jax.Array,
    B_w_up: jax.Array,
    B_w_down: jax.Array,
    gate_w: jax.Array,
):
    del B_x
    hbm = pl.BlockSpec(memory_space=pl.ANY)
    out = pl.pallas_call(
        _kernel,
        out_shape=jax.ShapeDtypeStruct((S, D), BF16),
        in_specs=[hbm] * 9,
        out_specs=hbm,
        scratch_shapes=[
            pltpu.VMEM((D,), BF16),
            pltpu.VMEM((D,), BF16),
            pltpu.VMEM((S, D), BF16),
            pltpu.VMEM((D, 3 * D), BF16),
            pltpu.VMEM((H, DH, DH), BF16),
            pltpu.VMEM((D, D), BF16),
            pltpu.VMEM((D, F), BF16),
            pltpu.VMEM((D, F), BF16),
            pltpu.VMEM((F, D), BF16),
            pltpu.VMEM((D // 2, D), U32),
            pltpu.VMEM((D // 2, D), U32),
            pltpu.VMEM((D // 2, D), U32),
            pltpu.VMEM((NP, AUG, 128), F32),
            pltpu.VMEM((NP, AUG // 2, 128), U32),
            pltpu.VMEM((2, T // 2, D), U32),
            pltpu.VMEM((S // 16, 128), F32),
            pltpu.VMEM((S, 128), F32),
            pltpu.VMEM((D, 128), F32),
            pltpu.VMEM((F, 128), F32),
            pltpu.VMEM((8, D), F32),
            pltpu.VMEM((NGATE, 16, D), BF16),
            pltpu.VMEM((S, D), BF16),
            pltpu.SemaphoreType.DMA((24 + NGATE,)),
            pltpu.SemaphoreType.DMA((4,)),
        ],
        compiler_params=pltpu.CompilerParams(vmem_limit_bytes=110 * 2**20),
    )(A_x.reshape(S, D), A_wqkv, A_w_phi, A_wo, B_w_r, B_w_gate, B_w_up, B_w_down, gate_w)
    return out.reshape(1, S, D)
```
